```python
import jax
import jax.numpy as jnp

def _softmax(x, axis=-1):
    return jax.nn.softmax(x, axis=axis)
def _gelu(x):
    return jax.nn.gelu(x, approximate=True)
def _silu(x):
    return jax.nn.silu(x)
def _sigmoid(x):
    return jax.nn.sigmoid(x)
def _layernorm(x, axis=-1, eps=1e-5):
    m = jnp.mean(x, axis=axis, keepdims=True)
    v = jnp.var(x, axis=axis, keepdims=True)
    return (x - m) / jnp.sqrt(v + eps)
def _scatter_add(tgt, idx, src, axis=0):
    return tgt.at[idx].add(src)
def _segment_sum(src, seg, n):
    return jax.ops.segment_sum(src, seg, n)
class _Rng:
    def __init__(self, key):
        self._k = key
    def _next(self):
        self._k, sub = jax.random.split(self._k)
        return sub
    def normal(self, shape):
        return jax.random.normal(self._next(), shape, dtype=jnp.bfloat16)
    def randint(self, lo, hi, shape):
        return jax.random.randint(self._next(), shape, lo, hi, dtype=jnp.int32)
    def uniform(self, shape, lo=0.0, hi=1.0):
        return jax.random.uniform(self._next(), shape, jnp.bfloat16, lo, hi)
    def permutation(self, n):
        return jax.random.permutation(self._next(), n)


kernel_name = 'interleave_layers__sliding_local_dilated__glu_gated_bilinear__prompt'

def setup_inputs():
    _rng = _Rng(jax.random.key(int.from_bytes(__import__("os").urandom(4), "little")))
    _w = (lambda a: (lambda t: t.astype(jnp.bfloat16) if jnp.issubdtype(t.dtype, jnp.floating) else t)(jnp.asarray(a)))
    def _A_setup():
        B, S, D = 1, 2048, 576
        return {
            "x": _w((lambda *s: _rng.normal(s) * 0.05)(B, S, D)),
            "wqkv": _w((lambda *s: _rng.normal(s) * 0.05)(D, 3 * D)),
            "wo": _w((lambda *s: _rng.normal(s) * 0.05)(D, D)),
        }
    _A_in = _A_setup()

    def _B_setup():
        B, S, D, F = 1, 2048, 576, 4608
        return {
            "x": _w((lambda *s: _rng.normal(s) * 0.05)(B, S, D)),
            "w_gate": _w((lambda *s: _rng.normal(s) * 0.05)(D, F) * (D ** -0.5)),
            "w_up": _w((lambda *s: _rng.normal(s) * 0.05)(D, F) * (D ** -0.5)),
            "w_down": _w((lambda *s: _rng.normal(s) * 0.05)(F, D) * (F ** -0.5)),
        }
    _B_in = _B_setup()

    return {
        "A_x": _A_in["x"],
        "A_wqkv": _A_in["wqkv"],
        "A_wo": _A_in["wo"],
        "B_x": _B_in["x"],
        "B_w_gate": _B_in["w_gate"],
        "B_w_up": _B_in["w_up"],
        "B_w_down": _B_in["w_down"],
    }

def reference(A_x, A_wqkv, A_wo, B_x, B_w_gate, B_w_up, B_w_down):
    def _A_ref(x, wqkv, wo):
        B, S, D = x.shape
        H = 32; Dh = D // H
        W, dil = 8, 2
        qkv = (lambda x, *d: x.transpose(*d))((x @ wqkv).reshape(B, S, 3, H, Dh), 2, 0, 3, 1, 4)
        q, k, v = qkv[0], qkv[1], qkv[2]
        scale = Dh ** -0.5
        pos = jnp.arange(S)
        off = jnp.arange(W) * dil
        idx = pos[:, None] - off[None, :]
        mask = idx >= 0
        idx_c = jnp.where(mask, idx, 0).reshape(-1)
        kg = k[:, :, idx_c, :].reshape(B, H, S, W, Dh)
        vg = v[:, :, idx_c, :].reshape(B, H, S, W, Dh)
        logits = jnp.einsum("bhsd,bhswd->bhsw", q, kg) * scale
        logits = jnp.where(mask[None, None, :, :], logits, -1e9)
        attn = _softmax(logits, axis=-1)
        o = jnp.einsum("bhsw,bhswd->bhsd", attn, vg)
        return (lambda x, *d: x.transpose(*d))(o, 0, 2, 1, 3).reshape(B, S, D) @ wo

    def _B_ref(x, w_gate, w_up, w_down):
        g = jnp.einsum("bsd,df->bsf", x, w_gate)
        u = jnp.einsum("bsd,df->bsf", x, w_up)
        h = g * u
        return jnp.einsum("bsf,fd->bsd", h, w_down)

    x = A_x
    x = x + _A_ref(_layernorm(x, axis=-1), A_wqkv, A_wo)
    x = x + _B_ref(_layernorm(x, axis=-1), B_w_gate, B_w_up, B_w_down)
    x = x + _A_ref(_layernorm(x, axis=-1), A_wqkv, A_wo)
    x = x + _B_ref(_layernorm(x, axis=-1), B_w_gate, B_w_up, B_w_down)
    return x
```

```python
import functools, numpy as np, jax, jax.numpy as jnp
from jax import lax
from jax.experimental import pallas as pl
from jax.experimental.pallas import tpu as pltpu
S, D, F = 2048, 576, 4608
H, DH, W, DIL = 32, 18, 8, 2
DP = 640; NT = 5; PADR = 16
HBM = pltpu.MemorySpace.HBM
f32, bf16 = jnp.float32, jnp.bfloat16
NTD = (((1,), (1,)), ((), ()))

def ln_T(xb):
    m = jnp.mean(xb, axis=0, keepdims=True)
    xc = xb - m
    v = jnp.mean(xc * xc, axis=0, keepdims=True)
    return xc * lax.rsqrt(v + 1e-5)

def make(MA=256, MB=512, FC=512, RC=32, doA=True, doB=True):
    nC = F // FC
    def kern(xT_hbm, wqkv_hbm, wo_hbm, wg_hbm, wu_hbm, wd_hbm, o_hbm,
             xin, wqkv, wo, wg, wu, wd, wp, woT, XT, ks, vs, qs, os_, xn_s, acc, sem, semc):
        c_qkv = pltpu.make_async_copy(wqkv_hbm, wqkv, sem.at[0])
        c_x = pltpu.make_async_copy(xT_hbm, xin, sem.at[1])
        c_wo = pltpu.make_async_copy(wo_hbm, wo, sem.at[2])
        c_qkv.start(); c_x.start(); c_wo.start()
        def ffn_cps(c):
            return [pltpu.make_async_copy(wg_hbm.at[:, pl.ds(c*FC, FC)], wg.at[c], semc.at[c]),
                    pltpu.make_async_copy(wu_hbm.at[:, pl.ds(c*FC, FC)], wu.at[c], semc.at[c]),
                    pltpu.make_async_copy(wd_hbm.at[:, pl.ds(c*FC, FC)], wd.at[c], semc.at[c])]
        for c in range(nC):
            for cp in ffn_cps(c): cp.start()
        r = lax.broadcasted_iota(jnp.int32, (DP, DP), 0)
        c_ = lax.broadcasted_iota(jnp.int32, (DP, DP), 1)
        src = jnp.where(c_ < D, (c_ & 31) * DH + (c_ >> 5), -1000)
        P0 = (r == src).astype(f32).astype(bf16)
        P1 = (r == src + 64).astype(f32).astype(bf16)
        ks[:, 0:PADR, :] = jnp.zeros((NT, PADR, 128), f32)
        vs[:, 0:PADR, :] = jnp.zeros((NT, PADR, 128), f32)
        c_qkv.wait()
        scale = DH ** -0.5
        wp[:, 0:DP] = jnp.dot(wqkv[:, 0:DP], P0, preferred_element_type=f32).astype(bf16)
        wp[:, DP:2*DP] = jnp.dot(wqkv[:, 512:1152], P1, preferred_element_type=f32).astype(bf16)
        wp[:, 2*DP:3*DP] = jnp.dot(wqkv[:, 1152:1728], P0[:D], preferred_element_type=f32).astype(bf16)
        c_wo.wait()
        woT[...] = jnp.dot(wo[...].astype(f32).T.astype(bf16), P0[:D], preferred_element_type=f32).astype(bf16)
        c_x.wait()
        XT[...] = xin[...].astype(f32)

        def a_blk(i, _):
            r0 = pl.multiple_of(i * MA, MA)
            xb = XT[:, pl.ds(r0, MA)]
            xn = ln_T(xb).T.astype(bf16)
            qkv = jnp.dot(xn, wp[...], preferred_element_type=f32)
            for t in range(NT):
                qs[t] = qkv[:, t*128:(t+1)*128] * scale
                ks[t, pl.ds(r0 + PADR, MA), :] = qkv[:, DP + t*128: DP + (t+1)*128]
                vs[t, pl.ds(r0 + PADR, MA), :] = qkv[:, 2*DP + t*128: 2*DP + (t+1)*128]
            for j in range(MA // RC):
                q = [qs[t, j*RC:(j+1)*RC, :] for t in range(NT)]
                ls = []
                for w in range(W):
                    st = r0 + (PADR + j*RC - DIL*w)
                    a = q[0] * ks[0, pl.ds(st, RC), :]
                    for t in range(1, NT):
                        a = a + q[t] * ks[t, pl.ds(st, RC), :]
                    a = a + pltpu.roll(a, 64, 1)
                    a = a + pltpu.roll(a, 32, 1)
                    if j * RC < DIL * w:
                        pos = r0 + j*RC + lax.broadcasted_iota(jnp.int32, (RC, 128), 0)
                        a = jnp.where(pos >= DIL*w, a, -1e9)
                    ls.append(a)
                m = functools.reduce(jnp.maximum, ls)
                ps = [jnp.exp(l - m) for l in ls]
                inv = 1.0 / functools.reduce(jnp.add, ps)
                for t in range(NT):
                    o = None
                    for w in range(W):
                        st = r0 + (PADR + j*RC - DIL*w)
                        pv = ps[w] * vs[t, pl.ds(st, RC), :]
                        o = pv if o is None else o + pv
                    os_[j*RC:(j+1)*RC, t*128:(t+1)*128] = (o * inv).astype(bf16)
            XT[:, pl.ds(r0, MA)] = xb + lax.dot_general(woT[...], os_[...], NTD, preferred_element_type=f32)

        def b_blk(layer, i, _):
            r0 = pl.multiple_of(i * MB, MB)
            xn_s[...] = ln_T(XT[:, pl.ds(r0, MB)]).T.astype(bf16)
            acc[...] = XT[:, pl.ds(r0, MB)]
            def ch(c, _):
                if layer == 0:
                    @pl.when(i == 0)
                    def _():
                        for cp in ffn_cps(c): cp.wait()
                xn = xn_s[...]
                g = jnp.dot(xn, wg[c], preferred_element_type=f32)
                u = jnp.dot(xn, wu[c], preferred_element_type=f32)
                h = (g * u).astype(bf16)
                acc[...] += lax.dot_general(wd[c], h, NTD, preferred_element_type=f32)
            lax.fori_loop(0, nC, ch, None)
            if layer == 0:
                XT[:, pl.ds(r0, MB)] = acc[...]
            else:
                xin[:, pl.ds(r0, MB)] = acc[...].astype(bf16)
                pltpu.make_async_copy(xin.at[:, pl.ds(r0, MB)], o_hbm.at[:, pl.ds(r0, MB)], sem.at[3]).start()

        for layer in range(2):
            if doA: lax.fori_loop(0, S // MA, a_blk, None)
            lax.fori_loop(0, S // MB, functools.partial(b_blk, layer), None)
        pltpu.make_async_copy(xin, o_hbm, sem.at[3]).wait()

    def fn(A_x, A_wqkv, A_wo, B_x, B_w_gate, B_w_up, B_w_down):
        o = pl.pallas_call(kern, out_shape=jax.ShapeDtypeStruct((D, S), bf16),
            in_specs=[pl.BlockSpec(memory_space=HBM)]*6,
            out_specs=pl.BlockSpec(memory_space=HBM),
            scratch_shapes=[pltpu.VMEM((D, S), bf16), pltpu.VMEM((D, 3*D), bf16), pltpu.VMEM((D, D), bf16),
                            pltpu.VMEM((nC, D, FC), bf16), pltpu.VMEM((nC, D, FC), bf16), pltpu.VMEM((nC, D, FC), bf16),
                            pltpu.VMEM((D, 3*DP), bf16), pltpu.VMEM((D, DP), bf16), pltpu.VMEM((D, S), f32),
                            pltpu.VMEM((NT, S+PADR, 128), f32), pltpu.VMEM((NT, S+PADR, 128), f32),
                            pltpu.VMEM((NT, MA, 128), f32), pltpu.VMEM((MA, DP), bf16),
                            pltpu.VMEM((MB, D), bf16), pltpu.VMEM((D, MB), f32),
                            pltpu.SemaphoreType.DMA((4,)), pltpu.SemaphoreType.DMA((nC,))],
            compiler_params=pltpu.CompilerParams(vmem_limit_bytes=100*1024*1024))(
                A_x[0].T, A_wqkv, A_wo, B_w_gate, B_w_up, B_w_down.T)
        return o.T[None]
    return fn


_fn = make()


@jax.jit
def pallas_interleave_layers__sliding_local_dilated__glu_gated_bilinear__prompt_kernel(
    A_x, A_wqkv, A_wo, B_x, B_w_gate, B_w_up, B_w_down):
    return _fn(A_x, A_wqkv, A_wo, B_x, B_w_gate, B_w_up, B_w_down)
```

```python
import functools
import jax
import jax.numpy as jnp
from jax import lax
from jax.experimental import pallas as pl
from jax.experimental.pallas import tpu as pltpu

S, D, F = 2048, 576, 4608
H, DH, W, DIL = 32, 18, 8, 2
NT, PADR = 5, 16
MA = 256
NB = S // MA
SH = S // 2
DHF = D // 2
HBM = pltpu.MemorySpace.HBM
f32, bf16 = jnp.float32, jnp.bfloat16
NTD = (((1,), (1,)), ((), ()))


def dot(a, b):
    return jnp.dot(a, b, preferred_element_type=f32)


def ntd(a, b):
    return lax.dot_general(a, b, NTD, preferred_element_type=f32)


def ln_T(xb):
    m = jnp.mean(xb, axis=0, keepdims=True)
    xc = xb - m
    v = jnp.mean(xc * xc, axis=0, keepdims=True)
    return xc * lax.rsqrt(v + 1e-5)


def lhs7(a11, a12, a21, a22):
    return [a11 + a22, a21 + a22, a11, a22, a11 + a12, a21 - a11, a12 - a22]


def rhs7(b11, b12, b21, b22):
    return [b11 + b22, b11, b12 - b22, b21 - b11, b22, b11 + b12, b21 + b22]


def out4(m):
    return (m[0] + m[3] - m[4] + m[6], m[2] + m[4], m[1] + m[3], m[0] - m[1] + m[2] + m[5])


def perm(nrow, ncol, shift, col0=0):
    r = lax.broadcasted_iota(jnp.int32, (nrow, ncol), 0)
    c = lax.broadcasted_iota(jnp.int32, (nrow, ncol), 1) + col0
    src = jnp.where(c < D, (c & 31) * DH + (c >> 5) + shift, -1)
    return jnp.where(r == src, 1.0, 0.0).astype(bf16)


def make(MH=1024, FC=512, RC=64, unroll_all=True, offs=(0.0, 0.5, 0.25), wo_first=False, sc=1.0):
    nC = F // FC
    FH = FC // 2
    nM = SH // MH
    PR = 256 // NB

    def kern(xT_hbm, wqkv_hbm, wo_hbm, wg_hbm, wu_hbm, wd_hbm, o_hbm,
             xin, wqkv, wo, wg, wu, wd, wp, woT, X, Y, xni, ks, vs, qs, os_,
             L, xr, wS, wr, wdS, acc, sem):
        c_qkv = pltpu.make_async_copy(wqkv_hbm, wqkv, sem.at[0])
        c_x = pltpu.make_async_copy(xT_hbm, xin, sem.at[1])
        c_wo = pltpu.make_async_copy(wo_hbm, wo, sem.at[2])
        c_ffn = [pltpu.make_async_copy(wg_hbm, wg, sem.at[4]),
                 pltpu.make_async_copy(wu_hbm, wu, sem.at[5]),
                 pltpu.make_async_copy(wd_hbm, wd, sem.at[6])]
        c_qkv.start(); c_x.start(); c_wo.start()
        for cp in c_ffn:
            cp.start()
        P0 = perm(640, 512, 0)
        P1 = perm(640, 512, 64)
        lane = lax.broadcasted_iota(jnp.int32, (1152, 128), 1)
        Pqk = jnp.where(lane < 64, perm(1152, 128, 0, 512), perm(1152, 128, D, 448))
        Pv4 = perm(D, 128, 0, 512)
        ks[:, 0:PADR, :] = jnp.zeros((NT, PADR, 128), f32)
        vs[:, 0:PADR, :] = jnp.zeros((NT, PADR, 128), f32)
        c_qkv.wait()
        wp[:, 0:512] = dot(wqkv[:, 0:640], P0).astype(bf16)
        wp[:, 512:1024] = dot(wqkv[:, 512:1152], P1).astype(bf16)
        wp[:, 1024:1536] = dot(wqkv[:, 1152:1728], P0[:D]).astype(bf16)
        wp[:, 1536:1664] = dot(wqkv[:, 0:1152], Pqk).astype(bf16)
        wp[:, 1664:1792] = dot(wqkv[:, 1152:1728], Pv4).astype(bf16)
        c_wo.wait()
        wot = wo[...].astype(f32).T.astype(bf16)
        woT[:, 0:512] = dot(wot, P0[:D]).astype(bf16)
        woT[:, 512:640] = dot(wot, Pv4).astype(bf16)
        c_x.wait()

        def tok(i, n=MA):
            return pl.ds(pl.multiple_of(i * n, n), n)

        def ffn_out(i):
            c11, c12, c21, c22 = out4([acc[k, :, tok(i, 128)] for k in range(7)])
            d = jnp.concatenate([jnp.concatenate([c11, c12], 1),
                                 jnp.concatenate([c21, c22], 1)], 0)
            return Y[:, tok(i)] + d

        def s1(layer, i):
            xb = xin[:, tok(i)].astype(f32) if layer == 0 else ffn_out(i)
            X[:, tok(i)] = xb
            xni[i % 2] = ln_T(xb).T.astype(bf16)

        def s2(i):
            scale = DH ** -0.5
            rows = pl.ds(pl.multiple_of(i * MA, MA) + PADR, MA)
            def part(g):
                r = dot(xni[i % 2], wp[:, g*512:(g+1)*512])
                for t in range(4):
                    v = r[:, t*128:(t+1)*128]
                    if g == 0:
                        qs[i % 2, t] = v * scale
                    else:
                        (ks if g == 1 else vs)[t, rows, :] = v
            def last():
                r = dot(xni[i % 2], wp[:, 1536:1792])
                qk4 = r[:, :128]
                lo = lax.broadcasted_iota(jnp.int32, (MA, 128), 1) < 64
                qs[i % 2, 4] = jnp.where(lo, qk4 * scale, 0.0)
                ks[4, rows, :] = jnp.where(lo, pltpu.roll(qk4, 64, 1), 0.0)
                vs[4, rows, :] = r[:, 128:]
            return [functools.partial(part, g) for g in range(3)] + [last]

        def s3(i):
            r0 = pl.multiple_of(i * MA, MA)
            def piece(j):
                q = [qs[i % 2, t, j*RC:(j+1)*RC, :] for t in range(NT)]
                ls = []
                for w in range(W):
                    st = r0 + (PADR + j*RC - DIL*w)
                    a = q[0] * ks[0, pl.ds(st, RC), :]
                    for t in range(1, NT):
                        a = a + q[t] * ks[t, pl.ds(st, RC), :]
                    a = a + pltpu.roll(a, 64, 1)
                    a = a + pltpu.roll(a, 32, 1)
                    if j * RC < DIL * w and (not isinstance(i, int) or i == 0):
                        pos = r0 + j*RC + lax.broadcasted_iota(jnp.int32, (RC, 128), 0)
                        a = jnp.where(pos >= DIL*w, a, -1e9)
                    ls.append(a)
                m = functools.reduce(jnp.maximum, ls)
                ps = [jnp.exp(l - m) for l in ls]
                inv = 1.0 / functools.reduce(jnp.add, ps)
                for t in range(NT):
                    o = None
                    for w in range(W):
                        st = r0 + (PADR + j*RC - DIL*w)
                        pv = ps[w] * vs[t, pl.ds(st, RC), :]
                        o = pv if o is None else o + pv
                    os_[i % 2, j*RC:(j+1)*RC, t*128:(t+1)*128] = (o * inv).astype(bf16)
            return [functools.partial(piece, j) for j in range(MA // RC)]

        def s4(i):
            Y[:, tok(i)] = X[:, tok(i)] + ntd(woT[...], os_[i % 2])

        def s5(i):
            xn = ln_T(Y[:, tok(i)]).T
            vals = lhs7(xn[:128, 0:256], xn[:128, 256:512], xn[128:, 0:256], xn[128:, 256:512])
            for k, v in enumerate(vals):
                L[k, tok(i, 128), :] = v.astype(bf16)
            xr[0, tok(i, 128), :] = xn[:128, 512:576].astype(bf16)
            xr[1, tok(i, 128), :] = xn[128:, 512:576].astype(bf16)

        def prep_up(p):
            r = tok(p, PR)
            r2 = pl.ds(pl.multiple_of(p * PR, PR) + 256, PR)
            def piece(c):
                cs = slice(c*FC, (c+1)*FC)
                vals = rhs7(wg[r, cs].astype(f32), wu[r, cs].astype(f32),
                            wg[r2, cs].astype(f32), wu[r2, cs].astype(f32))
                for k, v in enumerate(vals):
                    wS[c, k, r, :] = v.astype(bf16)
            return [functools.partial(piece, c) for c in range(nC)]

        def prep_dn(c, _):
            a, b = tok(2 * c, FH), tok(2 * c + 1, FH)
            vals = lhs7(wd[:DHF, a].astype(f32), wd[:DHF, b].astype(f32),
                        wd[DHF:, a].astype(f32), wd[DHF:, b].astype(f32))
            for k, v in enumerate(vals):
                wdS[c, k] = v.astype(bf16)
            wr[c, :, 0:FC] = wg[512:576, tok(c, FC)]
            wr[c, :, FC:] = wu[512:576, tok(c, FC)]

        def a_iter(layer, i, lo=None):
            ok = (lambda j: True) if lo is None else (lambda j: 0 <= j < NB)
            P = functools.partial
            mx, va, vb = [], [], []
            if ok(i + 1): mx += s2(i + 1)
            if ok(i - 1): mx.insert(0 if wo_first else len(mx), P(s4, i - 1))
            if ok(i): va += s3(i)
            if ok(i + 2): vb.append(P(s1, layer, i + 2))
            if ok(i - 2): vb.append(P(s5, i - 2))
            if layer == 0 and (lo is None or i >= 2):
                if unroll_all and i == 2:
                    for cp in c_ffn: cp.wait()
                vb = [P(prep_dn, i - 2, None)] + vb + prep_up(i - 2)
                if lo is not None and i == NB + 1:
                    vb += [P(prep_dn, c, None) for c in range(NB, nC)]
            items = []
            for off, lst in zip(offs, (mx, va, vb)):
                items += [((n + off) / len(lst) * (1.0 if lst is mx else sc), f) for n, f in enumerate(lst)]
            for _, f in sorted(items, key=lambda t: t[0]):
                f()

        def ffn_step(n, _):
            mb, c = n // nC, n % nC
            rows = tok(mb, MH)
            m = [dot(L[k, rows, :], wS[c, k]) for k in range(7)]
            r1 = dot(xr[0, rows, :], wr[c])
            r2 = dot(xr[1, rows, :], wr[c])
            g1, u1, g2, u2 = out4(m)
            h1 = (g1 + r1[:, :FC]) * (u1 + r1[:, FC:])
            h2 = (g2 + r2[:, :FC]) * (u2 + r2[:, FC:])
            vals = rhs7(h1[:, :FH], h2[:, :FH], h1[:, FH:], h2[:, FH:])
            for k, v in enumerate(vals):
                acc[k, :, rows] = jnp.where(c > 0, acc[k, :, rows], 0.0) + ntd(wdS[c, k], v.astype(bf16))

        for layer in range(2):
            if unroll_all:
                for i in range(-2, NB + 2):
                    a_iter(layer, i, 0)
            else:
                for i in range(-2, 2):
                    a_iter(layer, i, 0)
                if layer == 0:
                    for cp in c_ffn: cp.wait()
                lax.fori_loop(2, NB - 2, lambda i, _: a_iter(layer, i), None)
                for i in range(NB - 2, NB + 2):
                    a_iter(layer, i, 0)
            lax.fori_loop(0, nM * nC, ffn_step, None)

        def fin(i, _):
            xin[:, tok(i)] = ffn_out(i).astype(bf16)
            pltpu.make_async_copy(xin.at[:, tok(i)], o_hbm.at[:, tok(i)], sem.at[3]).start()
        lax.fori_loop(0, NB, fin, None)
        pltpu.make_async_copy(xin, o_hbm, sem.at[3]).wait()

    def fn(A_x, A_wqkv, A_wo, B_x, B_w_gate, B_w_up, B_w_down):
        V = pltpu.VMEM
        o = pl.pallas_call(
            kern, out_shape=jax.ShapeDtypeStruct((D, S), bf16),
            in_specs=[pl.BlockSpec(memory_space=HBM)] * 6,
            out_specs=pl.BlockSpec(memory_space=HBM),
            scratch_shapes=[V((D, S), bf16), V((D, 3*D), bf16), V((D, D), bf16),
                            V((D, F), bf16), V((D, F), bf16), V((D, F), bf16),
                            V((D, 1792), bf16), V((D, 640), bf16), V((D, S), f32), V((D, S), f32),
                            V((2, MA, D), bf16),
                            V((NT, S + PADR, 128), f32), V((NT, S + PADR, 128), f32),
                            V((2, NT, MA, 128), f32), V((2, MA, 640), bf16),
                            V((7, SH, 256), bf16), V((2, SH, 64), bf16),
                            V((nC, 7, 256, FC), bf16), V((nC, 64, 2*FC), bf16), V((nC, 7, DHF, FH), bf16),
                            V((7, DHF, SH), f32), pltpu.SemaphoreType.DMA((7,))],
            compiler_params=pltpu.CompilerParams(vmem_limit_bytes=120*1024*1024))(
                A_x[0].T, A_wqkv, A_wo, B_w_gate, B_w_up, B_w_down.T)
        return o.T[None]
    return fn


_fn = make()


@jax.jit
def pallas_interleave_layers__sliding_local_dilated__glu_gated_bilinear__prompt_kernel(
    A_x, A_wqkv, A_wo, B_x, B_w_gate, B_w_up, B_w_down):
    return _fn(A_x, A_wqkv, A_wo, B_x, B_w_gate, B_w_up, B_w_down)
```
